```python
import jax
import jax.numpy as jnp

def _softmax(x, axis=-1):
    return jax.nn.softmax(x, axis=axis)
def _gelu(x):
    return jax.nn.gelu(x, approximate=True)
def _silu(x):
    return jax.nn.silu(x)
def _sigmoid(x):
    return jax.nn.sigmoid(x)
def _layernorm(x, axis=-1, eps=1e-5):
    m = jnp.mean(x, axis=axis, keepdims=True)
    v = jnp.var(x, axis=axis, keepdims=True)
    return (x - m) / jnp.sqrt(v + eps)
def _scatter_add(tgt, idx, src, axis=0):
    return tgt.at[idx].add(src)
def _segment_sum(src, seg, n):
    return jax.ops.segment_sum(src, seg, n)
class _Rng:
    def __init__(self, key):
        self._k = key
    def _next(self):
        self._k, sub = jax.random.split(self._k)
        return sub
    def normal(self, shape):
        return jax.random.normal(self._next(), shape, dtype=jnp.bfloat16)
    def randint(self, lo, hi, shape):
        return jax.random.randint(self._next(), shape, lo, hi, dtype=jnp.int32)
    def uniform(self, shape, lo=0.0, hi=1.0):
        return jax.random.uniform(self._next(), shape, jnp.bfloat16, lo, hi)
    def permutation(self, n):
        return jax.random.permutation(self._next(), n)


kernel_name = 'standalone__convnext_block__vision'

def setup_inputs():
    _rng = _Rng(jax.random.key(int.from_bytes(__import__("os").urandom(4), "little")))
    _w = (lambda a: (lambda t: t.astype(jnp.bfloat16) if jnp.issubdtype(t.dtype, jnp.floating) else t)(jnp.asarray(a)))
    H = W = 512
    C = 96
    return {
        "x": _w((lambda *s: _rng.normal(s) * 0.05)(1, H, W, C)),
        "dw": _w((lambda *s: _rng.normal(s) * 0.05)(7, 7, C)),
        "w1": _w((lambda *s: _rng.normal(s) * 0.05)(C, 4 * C)),
        "w2": _w((lambda *s: _rng.normal(s) * 0.05)(4 * C, C)),
    }

def reference(x, dw, w1, w2):
    B, H, W, C = x.shape
    pad = 3
    xp = jnp.pad(x, ((0,0),(pad,pad),(pad,pad),(0,0)))
    out = jnp.zeros_like(x)
    for i in range(7):
        for j in range(7):
            out = out + xp[:, i:i+H, j:j+W, :] * dw[i, j][None, None, None, :]
    h = _layernorm(out, axis=-1)
    return x + _gelu(h @ w1) @ w2
```

```python
import math

import jax
import jax.numpy as jnp
from jax import lax
import jax.experimental.pallas as pl
import jax.experimental.pallas.tpu as pltpu

KS = 7
PAD = 3
G = 8
LANES = 128
NSLOT = 5
XS = 56
HS = 52
EPS = 1e-5

_A = math.sqrt(2.0 / math.pi)
_S = (_A * 0.044715) ** (1.0 / 3.0)


def make(order="a"):
    def kernel(x_hbm, dw_ref, w1_ref, w2t_ref, o_hbm,
               xbuf, obuf, t_ref, w1t_ref, w2s_ref, y_ref, p_ref, hn_ref, isem, osem):
        H, C, W = x_hbm.shape
        NT = W // LANES
        CP = C // 2
        NG = H // G
        xu = x_hbm.bitcast(jnp.uint32)
        xflat = xbuf.reshape(NSLOT, NT, G * XS, LANES)

        def in_copies(slot, row0, nrows, dst0):
            return [
                pltpu.make_async_copy(
                    xu.at[pl.ds(row0, nrows), :, pl.ds(t * LANES, LANES)],
                    xbuf.at[slot, t, pl.ds(dst0, nrows), pl.ds(0, CP), :],
                    isem.at[slot, t])
                for t in range(NT)
            ]

        first = lambda: in_copies(0, 0, PAD, G - PAD)
        full = lambda g: in_copies((g + 1) % NSLOT, g * G + PAD, G, 0)
        last = lambda: in_copies(NG % NSLOT, H - (G - PAD), G - PAD, 0)

        def out_copy(g):
            return pltpu.make_async_copy(obuf.at[g % 2], o_hbm.at[pl.ds(g * G, G)], osem.at[g % 2])

        for c in first() + full(0) + full(1) + full(2):
            c.start()
        xbuf[0, :, pl.ds(0, G - PAD), pl.ds(0, CP), :] = jnp.zeros((NT, G - PAD, CP, LANES), jnp.uint32)

        w1t_ref[...] = w1_ref[...].astype(jnp.float32).T.astype(jnp.bfloat16)
        w2s_ref[...] = w2t_ref[...]
        jj = lax.broadcasted_iota(jnp.int32, (KS, LANES), 0)
        kk = lax.broadcasted_iota(jnp.int32, (KS, LANES), 1)
        onehot = jnp.where(kk // (2 * G) == jj, 1.0, 0.0).astype(jnp.float32)
        for i in range(KS):
            d = lax.dot_general(dw_ref[i].astype(jnp.float32), onehot, (((0,), (0,)), ((), ())),
                                preferred_element_type=jnp.float32)
            y_ref[pl.ds(i * (C // 16), C // 16), :, pl.ds(0, LANES)] = d.reshape(C // 16, 16, LANES)
        m = lax.broadcasted_iota(jnp.int32, (4 * G, LANES), 0)
        k = lax.broadcasted_iota(jnp.int32, (4 * G, LANES), 1)
        tap = (k % (2 * G)) // 2 + (KS - 1) - m // 2
        tap = jnp.where((k % 2) == (m % 2), tap, -1)
        odd = (m % 2) == 1
        for p in range(CP):
            acc = jnp.zeros((4 * G, LANES), jnp.float32)
            for i in range(KS):
                blk, row = i * (C // 16) + (2 * p) // 16, (2 * p) % 16
                d0 = y_ref[blk, pl.ds(row, 1), pl.ds(0, LANES)]
                d1 = y_ref[blk, pl.ds(row + 1, 1), pl.ds(0, LANES)]
                acc = jnp.where(tap == i, jnp.where(odd, d1, d0), acc)
            t_ref[p] = acc.astype(jnp.bfloat16)
        p_ref[...] = jnp.zeros(p_ref.shape, jnp.float32)

        lane = lax.broadcasted_iota(jnp.int32, (G, LANES), 1)
        zero = jnp.zeros((G, LANES), jnp.uint32)

        def conv(slot, p, s1, s2):
            v = [xflat[slot, t, pl.ds(p, G, stride=XS), :] for t in range(NT)]
            rows = []
            for j in range(KS):
                d = j - PAD
                if d == 0:
                    rows.append(jnp.concatenate(v, axis=1))
                    continue
                r = [pltpu.roll(u, (-d) % LANES, 1) for u in v]
                if d > 0:
                    sh = [jnp.where(lane < LANES - d, r[t], r[t + 1] if t + 1 < NT else zero) for t in range(NT)]
                else:
                    sh = [jnp.where(lane < -d, r[t - 1] if t > 0 else zero, r[t]) for t in range(NT)]
                rows.append(jnp.concatenate(sh, axis=1))
            rhs = pltpu.bitcast(jnp.concatenate(rows, axis=0), jnp.bfloat16)
            res = jnp.dot(t_ref[p, :, pl.ds(0, KS * 2 * G)], rhs, preferred_element_type=jnp.float32)
            y = p_ref[p] + res[:2 * G]
            p_ref[p] = res[2 * G:]
            y_ref[p] = y
            if s1 is None:
                return y, y * y
            return s1 + y, s2 + y * y

        def norm(s1, s2):
            par = lax.broadcasted_iota(jnp.int32, s1.shape, 0) % 2

            def both(s):
                return s + jnp.where(par == 0, pltpu.roll(s, 2 * G - 1, 0), pltpu.roll(s, 1, 0))

            mean = both(s1) * (1.0 / C)
            var = jnp.maximum(both(s2) * (1.0 / C) - mean * mean, 0.0)
            rstd = lax.rsqrt(var + EPS) * _S
            for t in range(NT):
                ls = slice(t * LANES, (t + 1) * LANES)
                for p in range(CP):
                    hn = ((y_ref[p, :, ls] - mean[:, ls]) * rstd[:, ls]).astype(jnp.bfloat16)
                    hn_ref[t, pl.ds(p, G, stride=HS), :] = pltpu.bitcast(hn, jnp.uint32)

        def mlp_up(r):
            hb = jnp.concatenate([hn_ref[t, pl.ds(r * HS, CP), :] for t in range(NT)], axis=1)
            v = jnp.dot(w1t_ref[...], pltpu.bitcast(hb, jnp.bfloat16), preferred_element_type=jnp.float32)
            th = jnp.tanh(v * (v * v + _A / _S))
            return (v * th + v).astype(jnp.bfloat16)

        def mlp_down(g, r, act):
            o = jnp.dot(w2s_ref[...], act, preferred_element_type=jnp.float32)
            if r < PAD:
                slot, rr = g % NSLOT, r + G - PAD
            else:
                slot, rr = (g + 1) % NSLOT, r - PAD
            xr = jnp.concatenate([xbuf[slot, t, rr, pl.ds(0, CP), :] for t in range(NT)], axis=1)
            xr = pltpu.bitcast(xr, jnp.bfloat16).astype(jnp.float32)
            obuf[g % 2, r] = (xr + o * (0.5 / _S)).astype(jnp.bfloat16)

        for c in first() + full(0):
            c.wait()

        @pl.loop(0, 2)
        def _(s):
            s1 = s2 = None
            for p in range(CP):
                s1, s2 = conv(s, p, s1, s2)
            norm(s1, s2)

        @pl.loop(0, NG)
        def _(g):
            @pl.when(g + 3 < NG - 1)
            def _():
                for c in full(g + 3):
                    c.start()

            @pl.when(g + 3 == NG - 1)
            def _():
                for c in last():
                    c.start()
                xbuf[NG % NSLOT, :, pl.ds(G - PAD, PAD), pl.ds(0, CP), :] = jnp.zeros(
                    (NT, PAD, CP, LANES), jnp.uint32)

            @pl.when(g >= 2)
            def _():
                out_copy(g - 2).wait()

            @pl.when(g + 1 < NG - 1)
            def _():
                for c in full(g + 1):
                    c.wait()

            @pl.when(g + 1 == NG - 1)
            def _():
                for c in last():
                    c.wait()

            slot = (g + 2) % NSLOT
            s1 = s2 = None
            for r in range(G - 2):
                act = mlp_up(r)
                for p in range(r * 8, r * 8 + 8):
                    s1, s2 = conv(slot, p, s1, s2)
                mlp_down(g, r, act)
            a6 = mlp_up(G - 2)
            a7 = mlp_up(G - 1)
            norm(s1, s2)
            mlp_down(g, G - 2, a6)
            mlp_down(g, G - 1, a7)
            out_copy(g).start()

        out_copy(NG - 2).wait()
        out_copy(NG - 1).wait()

    def fn(x, dw, w1, w2):
        B, H, W, C = x.shape
        F = w1.shape[1]
        NT, CP = W // LANES, C // 2
        xt = jnp.transpose(x.reshape(H, W, C), (0, 2, 1))
        out = pl.pallas_call(
            kernel,
            out_shape=jax.ShapeDtypeStruct((H, C, W), x.dtype),
            in_specs=[pl.BlockSpec(memory_space=pl.ANY)] + [pl.BlockSpec(memory_space=pltpu.VMEM)] * 3,
            out_specs=pl.BlockSpec(memory_space=pl.ANY),
            scratch_shapes=[
                pltpu.VMEM((NSLOT, NT, G, XS, LANES), jnp.uint32),
                pltpu.VMEM((2, G, C, W), jnp.bfloat16),
                pltpu.VMEM((CP, 4 * G, LANES), jnp.bfloat16),
                pltpu.VMEM((F, C), jnp.bfloat16),
                pltpu.VMEM((C, F), jnp.bfloat16),
                pltpu.VMEM((CP, 2 * G, W), jnp.float32),
                pltpu.VMEM((CP, 2 * G, W), jnp.float32),
                pltpu.VMEM((NT, G * HS, LANES), jnp.uint32),
                pltpu.SemaphoreType.DMA((NSLOT, NT)),
                pltpu.SemaphoreType.DMA((2,)),
            ],
            compiler_params=pltpu.CompilerParams(vmem_limit_bytes=64 * 2**20),
            name="convnext",
        )(xt, dw, w1, w2.T)
        return jnp.transpose(out, (0, 2, 1)).reshape(B, H, W, C)

    return fn


_impl = make()


@jax.jit
def pallas_standalone__convnext_block__vision_kernel(x, dw, w1, w2):
    return _impl(x, dw, w1, w2)
```

```python
import math

import jax
import jax.numpy as jnp
from jax import lax
import jax.experimental.pallas as pl
import jax.experimental.pallas.tpu as pltpu

KS = 7
PAD = 3
G = 16
SUB = 8
LANES = 128
XS = 56
YS = 100
TOP = G - PAD
EPS = 1e-5

_A = math.sqrt(2.0 / math.pi)
_S = (_A * 0.044715) ** (1.0 / 3.0)


def _mm(a, b):
    return lax.dot_general(a, b, (((1,), (0,)), ((), ())), preferred_element_type=jnp.float32)


def _bf(v):
    return pltpu.bitcast(v, jnp.bfloat16)


def make(pat=(1, 2), flags=None, shift=8, f32h=True, PB=12, TR=4, NB=4, before=None, middle=None):
    def kernel(x_hbm, dw_hbm, w1_hbm, w2t_hbm, o_hbm,
               xbuf, obuf, dw_ref, w1_ref, w2t_ref, t_ref, w1t_ref, w2s_ref, d_ref, y_ref, p_ref, st_ref,
               wsem, isem, osem, tsem):
        H, C, W = x_hbm.shape
        NT = W // LANES
        CP = C // 2
        NG = H // G
        xu = x_hbm.bitcast(jnp.uint32)
        xflat = xbuf.reshape(NT, xbuf.shape[1] * XS, LANES)

        def in_copies(row0, nrows, s):
            return [
                pltpu.make_async_copy(
                    xu.at[pl.ds(row0, nrows), :, pl.ds(t * LANES, LANES)],
                    xbuf.at[t, pl.ds(row0 + TOP, nrows), pl.ds(0, CP), :],
                    isem.at[s, t])
                for t in range(NT)
            ]

        def start(copies):
            for c in copies:
                c.start()

        def wait(copies):
            for c in copies:
                c.wait()

        def out_copy(g):
            return pltpu.make_async_copy(obuf.at[g % 2], o_hbm.at[pl.ds(g * G, G)], osem.at[g % 2])

        BR = NB * G
        head = [in_copies(0, PAD, 0), in_copies(PAD, G, 1), in_copies(PAD + G, G, 2),
                in_copies(PAD + 2 * G, BR - 2 * G - PAD, 3)]
        block = lambda b: in_copies(b * BR, BR, 4)
        wcopies = [pltpu.make_async_copy(s, d, wsem.at[i]) for i, (s, d) in
                   enumerate(((dw_hbm, dw_ref), (w1_hbm, w1_ref), (w2t_hbm, w2t_ref)))]
        start(wcopies + head[0] + head[1])
        for r0, n in ((SUB, TOP - SUB), (H + TOP, PAD)):
            xbuf[:, pl.ds(r0, n), pl.ds(0, CP), :] = jnp.zeros((NT, n, CP, LANES), jnp.uint32)

        wait(wcopies)
        jj = lax.broadcasted_iota(jnp.int32, (KS, LANES), 0)
        kk = lax.broadcasted_iota(jnp.int32, (KS, LANES), 1)
        onehot = jnp.where(kk // G == jj, 1.0, 0.0).astype(jnp.float32)
        for i in range(KS):
            d_ref[i] = lax.dot_general(dw_ref[i].astype(jnp.float32), onehot, (((0,), (0,)), ((), ())),
                                       preferred_element_type=jnp.float32)
        w1f = w1_ref[...].astype(jnp.float32)
        w1f = jnp.concatenate([w1f, jnp.zeros((LANES - C, w1f.shape[1]), jnp.float32)], axis=0)
        w1t_ref[...] = pltpu.bitcast(w1f.T.astype(jnp.bfloat16), jnp.uint32)
        w2s_ref[...] = pltpu.bitcast(w2t_ref[...], jnp.uint32)
        q = lax.broadcasted_iota(jnp.int32, (3 * SUB, LANES), 0)
        k = lax.broadcasted_iota(jnp.int32, (3 * SUB, LANES), 1)
        tap = (k % G) // 2 + SUB * (k % 2) + (KS - 1) - q

        @pl.loop(0, C // SUB)
        def _(cb):
            for c in range(SUB):
                acc = jnp.zeros((3 * SUB, LANES), jnp.float32)
                for i in range(KS):
                    acc = jnp.where(tap == i, d_ref[i, pl.ds(cb * SUB + c, 1), :], acc)
                t_ref[cb * SUB + c] = acc

        lane = lax.broadcasted_iota(jnp.int32, (SUB, LANES), 1)
        zero = jnp.zeros((SUB, LANES), jnp.uint32)

        def shifts(v):
            rows = []
            for j in range(KS):
                d = j - PAD
                if d == 0:
                    rows.append(jnp.concatenate(v, axis=1))
                    continue
                r = [pltpu.roll(u, (-d) % LANES, 1) for u in v]
                if d > 0:
                    sh = [jnp.where(lane < LANES - d, r[t], r[t + 1] if t + 1 < NT else zero) for t in range(NT)]
                else:
                    sh = [jnp.where(lane < -d, r[t - 1] if t > 0 else zero, r[t]) for t in range(NT)]
                rows.append(jnp.concatenate(sh, axis=1))
            rows.append(jnp.zeros((SUB, W), jnp.uint32))
            return _bf(jnp.concatenate(rows, axis=0))

        def rows8(row0, p):
            return [xflat[t, pl.ds(row0 * XS + p, SUB, stride=XS), :] for t in range(NT)]

        def issue(gi, ps):
            out = []
            for p in ps:
                a = rows8((gi + 1) * G, p)
                b = rows8((gi + 1) * G + SUB, p)
                lo, hi = jnp.uint32(0xFFFF), jnp.uint32(0xFFFF0000)
                for c, v in ((2 * p, [(u & lo) | (w << 16) for u, w in zip(a, b)]),
                             (2 * p + 1, [(u >> 16) | (w & hi) for u, w in zip(a, b)])):
                    out.append((c, _mm(t_ref[c], shifts(v))))
            return out

        def commit(gi, results, first):
            if not results:
                return
            s = None
            for c, res in results:
                y = jnp.concatenate([p_ref[c] + res[:SUB], res[SUB:G]], axis=0)
                p_ref[c] = res[G:]
                for t in range(NT):
                    for hh in range(2):
                        y_ref[gi % 2, t, pl.ds(hh * SUB * YS + c, SUB, stride=YS), :] = (
                            y[hh * SUB:(hh + 1) * SUB, t * LANES:(t + 1) * LANES])
                s = (y, y * y) if s is None else (s[0] + y, s[1] + y * y)
            if first:
                st_ref[2], st_ref[3] = s
            else:
                st_ref[2] += s[0]
                st_ref[3] += s[1]

        def finish_stats():
            mean = st_ref[2] * (1.0 / C)
            var = jnp.maximum(st_ref[3] * (1.0 / C) - mean * mean, 0.0)
            st_ref[0] = mean
            st_ref[1] = lax.rsqrt(var + EPS) * _S

        def up(g, r0, r):
            off = r0 * YS if isinstance(r0, int) else pl.multiple_of(r0 * YS, SUB)
            y = jnp.concatenate([y_ref[g % 2, t, pl.ds(off + r * YS, C), :] for t in range(NT)], axis=1)
            h = (y - st_ref[0, pl.ds(r0 + r, 1), :]) * st_ref[1, pl.ds(r0 + r, 1), :]
            h = jnp.concatenate([h, jnp.zeros((LANES - C, W), jnp.float32)], axis=0)
            v = _mm(_bf(w1t_ref[...]), h if f32h else h.astype(jnp.bfloat16))
            th = jnp.tanh(v * (v * v + _A / _S))
            return (v * th + v).astype(jnp.bfloat16)

        def down(g, r, act):
            o = _mm(_bf(w2s_ref[...]), act)
            xr = jnp.concatenate([xbuf[t, g * G + TOP + r, pl.ds(0, CP), :] for t in range(NT)], axis=1)
            obuf[g % 2, r] = (_bf(xr).astype(jnp.float32) + o * (0.5 / _S)).astype(jnp.bfloat16)

        wait(head[0])

        @pl.loop(0, CP // PB)
        def _(pb):
            for i in range(PB):
                p = pb * PB + i
                even = lane % 2 == 0
                t0 = jnp.where(even, pltpu.roll(t_ref[2 * p, pl.ds(G, SUB)], LANES - 1, 1), 0.0)
                t1 = jnp.where(even, 0.0, t_ref[2 * p + 1, pl.ds(G, SUB)])
                res = _mm(jnp.concatenate([t0, t1], axis=0), shifts(rows8(SUB, p)))
                p_ref[2 * p] = res[:SUB]
                p_ref[2 * p + 1] = res[SUB:]

        wait(head[1])
        start(head[2] + head[3])
        st_ref[2] = jnp.zeros((G, W), jnp.float32)
        st_ref[3] = jnp.zeros((G, W), jnp.float32)

        @pl.loop(0, CP // PB)
        def _(pb):
            commit(0, issue(0, [pb * PB + i for i in range(PB)]), False)

        finish_stats()
        wait(head[2])

        bef = list(before) if before else [pat[0]] * G
        mid = list(middle) if middle else [pat[1]] * G
        if shift and not before:
            mid[shift] += bef[0]
            bef[0] = 0
        assert sum(bef) + sum(mid) == CP

        @pl.loop(0, NG - 1)
        def _(g):
            @pl.when(g >= 2)
            def _():
                out_copy(g - 2).wait()

            @pl.when(g == 1)
            def _():
                wait(head[3])

            @pl.when(jnp.logical_and(g % NB == NB - 2, g < NG - NB))
            def _():
                wait(block(g // NB + 1))

            @pl.when(jnp.logical_and(g % NB == 0, g < NG - NB))
            def _():
                start(block(g // NB + 1))

            p = 0
            for r in range(G):
                res = issue(g + 1, range(p, p + bef[r]))
                act = up(g, 0, r)
                commit(g + 1, res, p == 0)
                p += bef[r]
                commit(g + 1, issue(g + 1, range(p, p + mid[r])), p == 0)
                p += mid[r]
                if r == G - 1:
                    finish_stats()
                down(g, r, act)
            out_copy(g).start()

        g = NG - 1
        out_copy(g - 2).wait()

        def tail_copy(i):
            return pltpu.make_async_copy(obuf.at[g % 2, pl.ds(i * TR, TR)],
                                         o_hbm.at[pl.ds(g * G + i * TR, TR)], tsem.at[i])

        @pl.loop(0, G // TR)
        def _(i):
            act = up(g, i * TR, 0)
            for r in range(TR):
                nxt = up(g, i * TR, r + 1) if r + 1 < TR else None
                down(g, i * TR + r, act)
                act = nxt
            tail_copy(i).start()

        out_copy(g - 1).wait()
        for i in range(G // TR):
            tail_copy(i).wait()

    def fn(x, dw, w1, w2):
        B, H, W, C = x.shape
        F = w1.shape[1]
        NT, CP = W // LANES, C // 2
        xt = jnp.transpose(x.reshape(H, W, C), (0, 2, 1))
        out = pl.pallas_call(
            kernel,
            out_shape=jax.ShapeDtypeStruct((H, C, W), x.dtype),
            in_specs=[pl.BlockSpec(memory_space=pl.ANY)] * 4,
            out_specs=pl.BlockSpec(memory_space=pl.ANY),
            scratch_shapes=[
                pltpu.VMEM((NT, H + G, XS, LANES), jnp.uint32),
                pltpu.VMEM((2, G, C, W), jnp.bfloat16),
                pltpu.VMEM(dw.shape, dw.dtype),
                pltpu.VMEM((C, F), w1.dtype),
                pltpu.VMEM((C, F), w2.dtype),
                pltpu.VMEM((C, 3 * SUB, LANES), jnp.float32),
                pltpu.VMEM((F // 2, LANES), jnp.uint32),
                pltpu.VMEM((C // 2, F), jnp.uint32),
                pltpu.VMEM((KS, C, LANES), jnp.float32),
                pltpu.VMEM((2, NT, G * YS, LANES), jnp.float32),
                pltpu.VMEM((C, SUB, W), jnp.float32),
                pltpu.VMEM((4, G, W), jnp.float32),
                pltpu.SemaphoreType.DMA((3,)),
                pltpu.SemaphoreType.DMA((5, NT)),
                pltpu.SemaphoreType.DMA((2,)),
                pltpu.SemaphoreType.DMA((G // TR,)),
            ],
            compiler_params=pltpu.CompilerParams(vmem_limit_bytes=100 * 2**20, flags=flags),
            name="convnext",
        )(xt, dw, w1, w2.T)
        return jnp.transpose(out, (0, 2, 1)).reshape(B, H, W, C)

    return fn


_impl = make()


@jax.jit
def pallas_standalone__convnext_block__vision_kernel(x, dw, w1, w2):
    return _impl(x, dw, w1, w2)
```

```python
import math

import jax
import jax.numpy as jnp
from jax import lax
import jax.experimental.pallas as pl
import jax.experimental.pallas.tpu as pltpu

KS = 7
PAD = 3
G = 16
SUB = 8
LANES = 128
XS = 56
YS = 100
TOP = G - PAD
EPS = 1e-5

_A = math.sqrt(2.0 / math.pi)
_S = (_A * 0.044715) ** (1.0 / 3.0)


def _mm(a, b):
    return lax.dot_general(a, b, (((1,), (0,)), ((), ())), preferred_element_type=jnp.float32)


def _bf(v):
    return pltpu.bitcast(v, jnp.bfloat16)


def make(pat=(1, 2), flags=None, shift=8, f32h=True, PB=12, TR=4, NB=4, rev=True, nobc=False, before=None, middle=None):
    def kernel(x_hbm, dw_hbm, w1_hbm, w2t_hbm, o_hbm,
               xbuf, obuf, dw_ref, w1_ref, w2t_ref, t_ref, w1t_ref, w2s_ref, d_ref, y_ref, p_ref, st_ref,
               wsem, isem, osem, tsem):
        H, C, W = x_hbm.shape
        NT = W // LANES
        CP = C // 2
        NG = H // G
        xu = x_hbm.bitcast(jnp.uint32)
        xflat = xbuf.reshape(NT, xbuf.shape[1] * XS, LANES)

        def in_copies(row0, nrows, s):
            return [
                pltpu.make_async_copy(
                    xu.at[pl.ds(row0, nrows), :, pl.ds(t * LANES, LANES)],
                    xbuf.at[t, pl.ds(row0 + TOP, nrows), pl.ds(0, CP), :],
                    isem.at[s, t])
                for t in range(NT)
            ]

        def start(copies):
            for c in copies:
                c.start()

        def wait(copies):
            for c in copies:
                c.wait()

        def out_copy(g):
            return pltpu.make_async_copy(obuf.at[g & 1], o_hbm.at[pl.ds(g * G, G)], osem.at[g & 1])

        BR = NB * G
        head = [in_copies(0, PAD, 0), in_copies(PAD, G, 1), in_copies(PAD + G, G, 2)]
        NS = (H - 2 * G - PAD) // BR
        block = lambda b: in_copies(PAD + 2 * G + b * BR, BR, 3)
        rest = in_copies(PAD + 2 * G + NS * BR, H - (PAD + 2 * G + NS * BR), 3)
        wcopies = [pltpu.make_async_copy(s, d, wsem.at[i]) for i, (s, d) in
                   enumerate(((dw_hbm, dw_ref), (w1_hbm, w1_ref), (w2t_hbm, w2t_ref)))]
        start(wcopies + head[0] + head[1])
        for r0, n in ((SUB, TOP - SUB), (H + TOP, PAD)):
            xbuf[:, pl.ds(r0, n), pl.ds(0, CP), :] = jnp.zeros((NT, n, CP, LANES), jnp.uint32)

        wait(wcopies)
        jj = lax.broadcasted_iota(jnp.int32, (KS, LANES), 0)
        kk = lax.broadcasted_iota(jnp.int32, (KS, LANES), 1)
        onehot = jnp.where(kk // G == jj, 1.0, 0.0).astype(jnp.float32)
        for i in range(KS):
            d_ref[i] = lax.dot_general(dw_ref[i].astype(jnp.float32), onehot, (((0,), (0,)), ((), ())),
                                       preferred_element_type=jnp.float32)
        w1f = w1_ref[...].astype(jnp.float32)
        w1f = jnp.concatenate([w1f, jnp.zeros((LANES - C, w1f.shape[1]), jnp.float32)], axis=0)
        F = w1f.shape[1]
        order = [i // 8 * 8 + (7 - i % 8 if rev else i % 8) for i in range(F // 16)]
        flip = lambda m: jnp.concatenate([m[16 * i:16 * i + 16] for i in order], axis=0)
        w1t_ref[...] = pltpu.bitcast(flip(w1f.T).astype(jnp.bfloat16), jnp.uint32)
        w2s_ref[...] = pltpu.bitcast(w2t_ref[...], jnp.uint32)
        q = lax.broadcasted_iota(jnp.int32, (3 * SUB, LANES), 0)
        k = lax.broadcasted_iota(jnp.int32, (3 * SUB, LANES), 1)
        tap = (k % G) // 2 + SUB * (k % 2) + (KS - 1) - q

        @pl.loop(0, C // SUB)
        def _(cb):
            for c in range(SUB):
                acc = jnp.zeros((3 * SUB, LANES), jnp.float32)
                for i in range(KS):
                    acc = jnp.where(tap == i, d_ref[i, pl.ds(cb * SUB + c, 1), :], acc)
                t_ref[cb * SUB + c] = acc

        lane = lax.broadcasted_iota(jnp.int32, (SUB, LANES), 1)
        zero = jnp.zeros((SUB, LANES), jnp.uint32)

        def shifts(v):
            rows = []
            for j in range(KS):
                d = j - PAD
                if d == 0:
                    rows.append(jnp.concatenate(v, axis=1))
                    continue
                r = [pltpu.roll(u, (-d) % LANES, 1) for u in v]
                if d > 0:
                    sh = [jnp.where(lane < LANES - d, r[t], r[t + 1] if t + 1 < NT else zero) for t in range(NT)]
                else:
                    sh = [jnp.where(lane < -d, r[t - 1] if t > 0 else zero, r[t]) for t in range(NT)]
                rows.append(jnp.concatenate(sh, axis=1))
            rows.append(jnp.zeros((SUB, W), jnp.uint32))
            return _bf(jnp.concatenate(rows, axis=0))

        def rows8(row0, p):
            return [xflat[t, pl.ds(row0 * XS + p, SUB, stride=XS), :] for t in range(NT)]

        def issue(gi, ps):
            out = []
            for p in ps:
                a = rows8((gi + 1) * G, p)
                b = rows8((gi + 1) * G + SUB, p)
                lo, hi = jnp.uint32(0xFFFF), jnp.uint32(0xFFFF0000)
                for c, v in ((2 * p, [(u & lo) | (w << 16) for u, w in zip(a, b)]),
                             (2 * p + 1, [(u >> 16) | (w & hi) for u, w in zip(a, b)])):
                    out.append((c, _mm(t_ref[c], shifts(v))))
            return out

        def commit(gi, results, first):
            if not results:
                return
            s = None
            for c, res in results:
                y = jnp.concatenate([p_ref[c] + res[:SUB], res[SUB:G]], axis=0)
                p_ref[c] = res[G:]
                for t in range(NT):
                    for hh in range(2):
                        y_ref[gi & 1, t, pl.ds(hh * SUB * YS + c, SUB, stride=YS), :] = (
                            y[hh * SUB:(hh + 1) * SUB, t * LANES:(t + 1) * LANES])
                s = (y, y * y) if s is None else (s[0] + y, s[1] + y * y)
            if first:
                st_ref[2], st_ref[3] = s
            else:
                st_ref[2] += s[0]
                st_ref[3] += s[1]

        def finish_stats():
            mean = st_ref[2] * (1.0 / C)
            var = jnp.maximum(st_ref[3] * (1.0 / C) - mean * mean, 0.0)
            st_ref[0] = mean
            st_ref[1] = lax.rsqrt(var + EPS) * _S

        def up(g, r0, r):
            off = r0 * YS if isinstance(r0, int) else pl.multiple_of(r0 * YS, SUB)
            y = jnp.concatenate([y_ref[g & 1, t, pl.ds(off + r * YS, C), :] for t in range(NT)], axis=1)
            h = (y - st_ref[0, pl.ds(r0 + r, 1), :]) * st_ref[1, pl.ds(r0 + r, 1), :]
            h = jnp.concatenate([h, jnp.zeros((LANES - C, W), jnp.float32)], axis=0)
            v = _mm(_bf(w1t_ref[...]), h if f32h else h.astype(jnp.bfloat16))
            th = jnp.tanh(v * (v * v + _A / _S))
            return flip(v * th + v).astype(jnp.bfloat16)

        def down(g, r, act):
            o = _mm(_bf(w2s_ref[...]), act)
            xr = jnp.concatenate([xbuf[t, g * G + TOP + r, pl.ds(0, CP), :] for t in range(NT)], axis=1)
            obuf[g & 1, r] = (_bf(xr).astype(jnp.float32) + o * (0.5 / _S)).astype(jnp.bfloat16)

        wait(head[0])

        @pl.loop(0, CP // PB)
        def _(pb):
            for i in range(PB):
                p = pb * PB + i
                even = lane % 2 == 0
                t0 = jnp.where(even, pltpu.roll(t_ref[2 * p, pl.ds(G, SUB)], LANES - 1, 1), 0.0)
                t1 = jnp.where(even, 0.0, t_ref[2 * p + 1, pl.ds(G, SUB)])
                res = _mm(jnp.concatenate([t0, t1], axis=0), shifts(rows8(SUB, p)))
                p_ref[2 * p] = res[:SUB]
                p_ref[2 * p + 1] = res[SUB:]

        wait(head[1])
        start(head[2])
        st_ref[2] = jnp.zeros((G, W), jnp.float32)
        st_ref[3] = jnp.zeros((G, W), jnp.float32)

        @pl.loop(0, CP // PB)
        def _(pb):
            commit(0, issue(0, [pb * PB + i for i in range(PB)]), False)

        finish_stats()
        wait(head[2])

        bef = list(before) if before else [pat[0]] * G
        mid = list(middle) if middle else [pat[1]] * G
        if shift and not before:
            mid[shift] += bef[0]
            bef[0] = 0
        assert sum(bef) + sum(mid) == CP

        def step(g):
            @pl.when(g >= 2)
            def _():
                out_copy(g - 2).wait()

            p = 0
            for r in range(G):
                res = issue(g + 1, range(p, p + bef[r]))
                act = up(g, 0, r)
                commit(g + 1, res, p == 0)
                p += bef[r]
                commit(g + 1, issue(g + 1, range(p, p + mid[r])), p == 0)
                p += mid[r]
                if r == G - 1:
                    finish_stats()
                down(g, r, act)
            out_copy(g).start()

        @pl.loop(0, NS + 2)
        def _(s):
            pl.when(s < NS)(lambda: start(block(s)))
            pl.when(s == NS)(lambda: start(rest))
            pl.loop(jnp.maximum((s - 1) * NB + 1, 0), jnp.minimum(s * NB + 1, NG - 1))(step)
            pl.when(s < NS)(lambda: wait(block(s)))
            pl.when(s == NS)(lambda: wait(rest))

        g = NG - 1
        out_copy(g - 2).wait()

        def tail_copy(i):
            return pltpu.make_async_copy(obuf.at[g & 1, pl.ds(i * TR, TR)],
                                         o_hbm.at[pl.ds(g * G + i * TR, TR)], tsem.at[i])

        @pl.loop(0, G // TR)
        def _(i):
            act = up(g, i * TR, 0)
            for r in range(TR):
                nxt = up(g, i * TR, r + 1) if r + 1 < TR else None
                down(g, i * TR + r, act)
                act = nxt
            tail_copy(i).start()

        out_copy(g - 1).wait()
        for i in range(G // TR):
            tail_copy(i).wait()

    def fn(x, dw, w1, w2):
        B, H, W, C = x.shape
        F = w1.shape[1]
        NT, CP = W // LANES, C // 2
        xt = jnp.transpose(x.reshape(H, W, C), (0, 2, 1))
        out = pl.pallas_call(
            kernel,
            out_shape=jax.ShapeDtypeStruct((H, C, W), x.dtype),
            in_specs=[pl.BlockSpec(memory_space=pl.ANY)] * 4,
            out_specs=pl.BlockSpec(memory_space=pl.ANY),
            scratch_shapes=[
                pltpu.VMEM((NT, H + G, XS, LANES), jnp.uint32),
                pltpu.VMEM((2, G, C, W), jnp.bfloat16),
                pltpu.VMEM(dw.shape, dw.dtype),
                pltpu.VMEM((C, F), w1.dtype),
                pltpu.VMEM((C, F), w2.dtype),
                pltpu.VMEM((C, 3 * SUB, LANES), jnp.float32),
                pltpu.VMEM((F // 2, LANES), jnp.uint32),
                pltpu.VMEM((C // 2, F), jnp.uint32),
                pltpu.VMEM((KS, C, LANES), jnp.float32),
                pltpu.VMEM((2, NT, G * YS, LANES), jnp.float32),
                pltpu.VMEM((C, SUB, W), jnp.float32),
                pltpu.VMEM((4, G, W), jnp.float32),
                pltpu.SemaphoreType.DMA((3,)),
                pltpu.SemaphoreType.DMA((4, NT)),
                pltpu.SemaphoreType.DMA((2,)),
                pltpu.SemaphoreType.DMA((G // TR,)),
            ],
            compiler_params=pltpu.CompilerParams(vmem_limit_bytes=100 * 2**20, flags=flags, disable_bounds_checks=nobc),
            name="convnext",
        )(xt, dw, w1, w2.T)
        return jnp.transpose(out, (0, 2, 1)).reshape(B, H, W, C)

    return fn


_impl = make()


@jax.jit
def pallas_standalone__convnext_block__vision_kernel(x, dw, w1, w2):
    return _impl(x, dw, w1, w2)
```

```python
import math

import jax
import jax.numpy as jnp
from jax import lax
import jax.experimental.pallas as pl
import jax.experimental.pallas.tpu as pltpu

KS = 7
PAD = 3
SUB = 8
LANES = 128
G = 18
M = G + KS - 1
XS = 56
YS = 100
TOP = 2 * SUB - PAD
EPS = 1e-5

_A = math.sqrt(2.0 / math.pi)
_S = (_A * 0.044715) ** (1.0 / 3.0)


def _mm(a, b):
    return lax.dot_general(a, b, (((1,), (0,)), ((), ())), preferred_element_type=jnp.float32)


def _bf(v):
    return pltpu.bitcast(v, jnp.bfloat16)


def make(flags=None, f32h=True, PB=24, TR=4, NB=4, dup=False, before=None, middle=None):
    bef = before or [0] + [2] * (G - 1)
    mid = middle or [4, 3] * 8 + [3, 3]

    def kernel(x_hbm, dw_hbm, w1_hbm, w2t_hbm, o_hbm,
               xbuf, obuf, dw_ref, w1_ref, w2t_ref, t_ref, w1t_ref, w2s_ref, d_ref, y_ref, p_ref, st_ref, e_ref,
               wsem, isem, osem, tsem):
        H, C, W = x_hbm.shape
        NT = W // LANES
        CP = C // 2
        NG = H // G
        xu = x_hbm.bitcast(jnp.uint32)
        xflat = xbuf.reshape(NT, xbuf.shape[1] * XS, LANES)

        def in_copies(row0, nrows, s):
            return [
                pltpu.make_async_copy(
                    xu.at[pl.ds(row0, nrows), :, pl.ds(t * LANES, LANES)],
                    xbuf.at[t, pl.ds(row0 + TOP, nrows), pl.ds(0, CP), :],
                    isem.at[s, t])
                for t in range(NT)
            ]

        def start(copies):
            for c in copies:
                c.start()

        def wait(copies):
            for c in copies:
                c.wait()

        def out_copy(g):
            return pltpu.make_async_copy(obuf.at[g & 1], o_hbm.at[pl.ds(g * G, G)], osem.at[g & 1])

        BR = NB * G
        R0 = PAD + 2
        head = [in_copies(0, R0, 0), in_copies(R0, G, 1), in_copies(R0 + G, G, 2)]
        NS = (H - 2 * G - R0) // BR
        block = lambda b: in_copies(R0 + 2 * G + b * BR, BR, 3)
        rest = in_copies(R0 + 2 * G + NS * BR, H - (R0 + 2 * G + NS * BR), 3)
        wcopies = [pltpu.make_async_copy(s, d, wsem.at[i]) for i, (s, d) in
                   enumerate(((dw_hbm, dw_ref), (w1_hbm, w1_ref), (w2t_hbm, w2t_ref)))]
        start(wcopies + head[0] + head[1])
        for r0, n in ((SUB, TOP - SUB), (H + TOP, (NG + 1) * G + R0 - H)):
            xbuf[:, pl.ds(r0, n), pl.ds(0, CP), :] = jnp.zeros((NT, n, CP, LANES), jnp.uint32)

        wait(wcopies)
        KM = 2 * SUB * KS
        jj = lax.broadcasted_iota(jnp.int32, (KS, LANES), 0)
        kk = lax.broadcasted_iota(jnp.int32, (KS, LANES), 1)
        col = jnp.where(kk < KM, kk // (2 * SUB), KS - 1 - (kk - KM) // 2)
        onehot = jnp.where(col == jj, 1.0, 0.0).astype(jnp.float32)
        for i in range(KS):
            d_ref[i] = lax.dot_general(dw_ref[i].astype(jnp.float32), onehot, (((0,), (0,)), ((), ())),
                                       preferred_element_type=jnp.float32)
        w1f = w1_ref[...].astype(jnp.float32)
        w1f = jnp.concatenate([w1f, jnp.zeros((LANES - C, w1f.shape[1]), jnp.float32)], axis=0)
        F = w1f.shape[1]
        order = [i // 8 * 8 + 7 - i % 8 for i in range(F // 16)]
        flip = lambda m: jnp.concatenate([m[16 * i:16 * i + 16] for i in order], axis=0)
        w1t_ref[...] = pltpu.bitcast(flip(w1f.T).astype(jnp.bfloat16), jnp.uint32)
        w2s_ref[...] = pltpu.bitcast(w2t_ref[...], jnp.uint32)

        def toeplitz(tap, c):
            acc = jnp.zeros(tap.shape, jnp.float32)
            for i in range(KS):
                acc = jnp.where(tap == i, d_ref[i, pl.ds(c, 1), :], acc)
            return acc

        lane = lax.broadcasted_iota(jnp.int32, (SUB, LANES), 1)
        sub = lax.broadcasted_iota(jnp.int32, (SUB, LANES), 0)
        zero = jnp.zeros((SUB, LANES), jnp.uint32)

        def shifts(v, extra):
            prev = lambda u, t: u[t - 1] if t > 0 else zero
            nxt = lambda u, t: u[t + 1] if t + 1 < NT else zero
            rows = []
            for j in range(KS):
                d = j - PAD
                if d == 0:
                    rows.append(jnp.concatenate(v, axis=1))
                    continue
                r = [pltpu.roll(u, (-d) % LANES, 1) for u in v]
                if d > 0:
                    sh = [jnp.where(lane < LANES - d, r[t], nxt(r, t)) for t in range(NT)]
                else:
                    sh = [jnp.where(lane < -d, prev(r, t), r[t]) for t in range(NT)]
                rows.append(jnp.concatenate(sh, axis=1))
            if extra is None:
                rows.append(jnp.zeros((SUB, W), jnp.uint32))
            else:
                d, src = PAD - sub, (lane + PAD) % LANES
                e = [jnp.broadcast_to(u, (SUB, LANES)) for u in extra]
                e = [jnp.where(src < d, nxt(e, t), jnp.where(src >= LANES + d, prev(e, t), e[t]))
                     for t in range(NT)]
                rows.append(jnp.concatenate(
                    [pltpu.roll(u, 0, 1, stride=1, stride_axis=0) for u in e], axis=1))
            return _bf(jnp.concatenate(rows, axis=0))

        def rows8(row0, p):
            return [xflat[t, pl.ds(row0 * XS + p, SUB, stride=XS), :] for t in range(NT)]

        lo = lambda a, b: [(u & jnp.uint32(0xFFFF)) | (w << 16) for u, w in zip(a, b)]
        hi = lambda a, b: [(u >> 16) | (w & jnp.uint32(0xFFFF0000)) for u, w in zip(a, b)]

        def lead(gi, p):
            r0 = gi * G + PAD + TOP
            ea, eb = ([xbuf[t, r0 + e, pl.ds(p, SUB), :] for t in range(NT)] for e in range(2))
            for e, f in enumerate((lo, hi)):
                for t, u in enumerate(f(ea, eb)):
                    e_ref[e, t, pl.ds(p, SUB), :] = pltpu.roll(u, LANES - PAD, 1)

        def issue(gi, p0, cs):
            out = []
            r0 = gi * G + PAD + TOP + 2
            for c in cs:
                i, e = divmod(c, 2)
                p = p0 + i
                if e == 0 or not out:
                    a, b = rows8(r0, p), rows8(r0 + SUB, p)
                extra = [e_ref[e, t, pl.ds(p, 1), :] for t in range(NT)]
                out.append((2 * p + e, _mm(t_ref[2 * p + e], shifts((lo, hi)[e](a, b), extra))))
                if c % (2 * SUB) == 2 * SUB - 1:
                    lead(gi + 1, p - (SUB - 1))
            return out

        def commit(gi, results, first):
            if not results:
                return
            s = None
            carried = lax.broadcasted_iota(jnp.int32, (SUB, W), 0) >= 2
            for c, res in results:
                y = jnp.concatenate([p_ref[c] + res[:SUB], res[SUB:]], axis=0)
                p_ref[c] = jnp.where(carried, res[2 * SUB:], 0.0)
                for t in range(NT):
                    for m0, r0, n in ((0, 0, SUB), (SUB, SUB, SUB), (2 * SUB, 2 * SUB, 2)):
                        y_ref[gi & 1, t, pl.ds(r0 * YS + c, n, stride=YS), :] = (
                            y[m0:m0 + n, t * LANES:(t + 1) * LANES])
                s = (y, y * y) if s is None else (s[0] + y, s[1] + y * y)
            if first:
                st_ref[2], st_ref[3] = s
            else:
                st_ref[2] += s[0]
                st_ref[3] += s[1]

        def finish_stats():
            mean = st_ref[2] * (1.0 / C)
            var = jnp.maximum(st_ref[3] * (1.0 / C) - mean * mean, 0.0)
            st_ref[0] = mean
            st_ref[1] = lax.rsqrt(var + EPS) * _S

        def up(g, r):
            m = (r + 2) % SUB if r < SUB else r
            y = jnp.concatenate([y_ref[g & 1, t, pl.ds(m * YS, C), :] for t in range(NT)], axis=1)
            h = (y - st_ref[0, pl.ds(m, 1), :]) * st_ref[1, pl.ds(m, 1), :]
            h = jnp.concatenate([h, jnp.zeros((LANES - C, W), jnp.float32)], axis=0)
            v = _mm(_bf(w1t_ref[...]), h if f32h else h.astype(jnp.bfloat16))
            th = jnp.tanh(v * (v * v + _A / _S))
            return flip(v * th + v).astype(jnp.bfloat16)

        def down(g, r, act):
            o = _mm(_bf(w2s_ref[...]), act)
            xr = jnp.concatenate([xbuf[t, g * G + TOP + r, pl.ds(0, CP), :] for t in range(NT)], axis=1)
            obuf[g & 1, r] = (_bf(xr).astype(jnp.float32) + o * (0.5 / _S)).astype(jnp.bfloat16)

        wait(head[0])
        for p in range(0, CP, SUB):
            lead(0, p)
        m = lax.broadcasted_iota(jnp.int32, (M, LANES), 0)
        k = lax.broadcasted_iota(jnp.int32, (M, LANES), 1)
        q = jnp.where(m < SUB, (m + SUB - 2) % SUB, m)
        rin = jnp.where(k < KM, (k % (2 * SUB)) // 2 + SUB * (k % 2) + 2, k % 2)
        tap = rin + (KS - 1) - q
        s_ = (lane % (2 * SUB)) // 2
        tap0 = s_ % 4 - 1 - (sub + SUB - 2) % SUB + PAD
        who = (1 - s_ // 4) * 2 + lane % 2

        @pl.loop(0, CP // PB)
        def _(pb):
            for i in range(0, PB, 2):
                p = pb * PB + i
                for e in range(4):
                    t_ref[2 * p + e] = toeplitz(tap, 2 * p + e)
                t1 = jnp.concatenate([jnp.where(who == e, toeplitz(tap0, 2 * p + e), 0.0) for e in range(4)], axis=0)
                v = [a | pltpu.roll(b, SUB // 2, 0) for a, b in zip(rows8(SUB, p), rows8(SUB, p + 1))]
                res = _mm(t1, shifts(v, None))
                for e in range(4):
                    p_ref[2 * p + e] = res[e * SUB:(e + 1) * SUB]

        wait(head[1])
        start(head[2])
        st_ref[2] = jnp.zeros((M, W), jnp.float32)
        st_ref[3] = jnp.zeros((M, W), jnp.float32)

        @pl.loop(0, CP // PB)
        def _(pb):
            commit(0, issue(0, pl.multiple_of(pb * PB, SUB), range(2 * PB)), False)

        finish_stats()
        wait(head[2])
        assert sum(bef) + sum(mid) == C

        def step(g):
            if dup:
                pl.when((g & 1) == 0)(lambda: step1(g, 0))
                pl.when((g & 1) == 1)(lambda: step1(g, 1))
            else:
                step1(g, g)

        def step1(g, par):
            @pl.when(g >= 2)
            def _():
                out_copy(g - 2).wait()

            p = 0
            for r in range(G):
                res = issue(g + 1, 0, range(p, p + bef[r]))
                act = up(par, r)
                commit(par + 1, res, p == 0)
                p += bef[r]
                commit(par + 1, issue(g + 1, 0, range(p, p + mid[r])), p == 0)
                p += mid[r]
                if r == G - 1:
                    finish_stats()
                down(g, r, act)
            out_copy(g).start()

        @pl.loop(0, NS + 2)
        def _(s):
            pl.when(s < NS)(lambda: start(block(s)))
            pl.when(s == NS)(lambda: start(rest))
            pl.loop(jnp.maximum((s - 1) * NB + 1, 0), jnp.minimum(s * NB + 1, NG))(step)
            pl.when(s < NS)(lambda: wait(block(s)))
            pl.when(s == NS)(lambda: wait(rest))

        g = NG
        NR = (H - NG * G) // TR
        out_copy(g - 2).wait()

        def tail_copy(i):
            return pltpu.make_async_copy(obuf.at[g & 1, pl.ds(i * TR, TR)],
                                         o_hbm.at[pl.ds(g * G + i * TR, TR)], tsem.at[i])

        for i in range(NR):
            act = up(g, i * TR)
            for r in range(TR):
                nxt = up(g, i * TR + r + 1) if r + 1 < TR else None
                down(g, i * TR + r, act)
                act = nxt
            tail_copy(i).start()

        out_copy(g - 1).wait()
        for i in range(NR):
            tail_copy(i).wait()

    def fn(x, dw, w1, w2):
        B, H, W, C = x.shape
        F = w1.shape[1]
        NT, CP = W // LANES, C // 2
        xt = jnp.transpose(x.reshape(H, W, C), (0, 2, 1))
        out = pl.pallas_call(
            kernel,
            out_shape=jax.ShapeDtypeStruct((H, C, W), x.dtype),
            in_specs=[pl.BlockSpec(memory_space=pl.ANY)] * 4,
            out_specs=pl.BlockSpec(memory_space=pl.ANY),
            scratch_shapes=[
                pltpu.VMEM((NT, (H // G + 1) * G + PAD + TOP + 3, XS, LANES), jnp.uint32),
                pltpu.VMEM((2, G, C, W), jnp.bfloat16),
                pltpu.VMEM(dw.shape, dw.dtype),
                pltpu.VMEM((C, F), w1.dtype),
                pltpu.VMEM((C, F), w2.dtype),
                pltpu.VMEM((C, M, LANES), jnp.float32),
                pltpu.VMEM((F // 2, LANES), jnp.uint32),
                pltpu.VMEM((C // 2, F), jnp.uint32),
                pltpu.VMEM((KS, C, LANES), jnp.float32),
                pltpu.VMEM((2, NT, (G + 2) * YS, LANES), jnp.float32),
                pltpu.VMEM((C, SUB, W), jnp.float32),
                pltpu.VMEM((4, M, W), jnp.float32),
                pltpu.VMEM((2, NT, CP, LANES), jnp.uint32),
                pltpu.SemaphoreType.DMA((3,)),
                pltpu.SemaphoreType.DMA((4, NT)),
                pltpu.SemaphoreType.DMA((2,)),
                pltpu.SemaphoreType.DMA((H % G // TR,)),
            ],
            compiler_params=pltpu.CompilerParams(vmem_limit_bytes=100 * 2**20, flags=flags),
            name="convnext",
        )(xt, dw, w1, w2.T)
        return jnp.transpose(out, (0, 2, 1)).reshape(B, H, W, C)

    return fn


_impl = make()


@jax.jit
def pallas_standalone__convnext_block__vision_kernel(x, dw, w1, w2):
    return _impl(x, dw, w1, w2)
```

```python
import math

import jax
import jax.numpy as jnp
from jax import lax
import jax.experimental.pallas as pl
import jax.experimental.pallas.tpu as pltpu

KS = 7
PAD = KS // 2
SUB = 8
LANES = 128
G = 2 * SUB + 2
M = G + KS - 1
KM = 2 * SUB * KS
XS = 56
YS = 100
TOP = 2 * SUB - PAD
NB = 4
TR = 4
EPS = 1e-5

CONV_BEFORE = (0,) + (2,) * (G - 1)
CONV_AFTER = (4, 3) * 8 + (3, 3)

_A = math.sqrt(2.0 / math.pi)
_S = (_A * 0.044715) ** (1.0 / 3.0)


def _mm(a, b):
    return lax.dot_general(a, b, (((1,), (0,)), ((), ())), preferred_element_type=jnp.float32)


def _bf16(words):
    return pltpu.bitcast(words, jnp.bfloat16)


def _iota(shape, axis):
    return lax.broadcasted_iota(jnp.int32, shape, axis)


def _start(copies):
    for c in copies:
        c.start()


def _wait(copies):
    for c in copies:
        c.wait()


def _low_halves(a, b):
    return [(u & jnp.uint32(0xFFFF)) | (w << 16) for u, w in zip(a, b)]


def _high_halves(a, b):
    return [(u >> 16) | (w & jnp.uint32(0xFFFF0000)) for u, w in zip(a, b)]


def _flip(m):
    order = [i // 8 * 8 + 7 - i % 8 for i in range(m.shape[0] // 16)]
    return jnp.concatenate([m[16 * i:16 * (i + 1)] for i in order], axis=0)


def _kernel(x_hbm, dw_hbm, w1_hbm, w2t_hbm, o_hbm,
            xbuf, obuf, dw_buf, w1_buf, w2t_buf, w1t_ref, w2t_ref, taps_ref, band_ref,
            lead_ref, y_ref, carry_ref, stat_ref, wsem, isem, osem):
    H, C, W = x_hbm.shape
    NT = W // LANES
    CP = C // 2
    NG = H // G
    x_words = x_hbm.bitcast(jnp.uint32)
    xflat = xbuf.reshape(NT, xbuf.shape[1] * XS, LANES)

    def in_copies(row0, nrows, s):
        return [
            pltpu.make_async_copy(
                x_words.at[pl.ds(row0, nrows), :, pl.ds(t * LANES, LANES)],
                xbuf.at[t, pl.ds(row0 + TOP, nrows), pl.ds(0, CP), :],
                isem.at[s, t])
            for t in range(NT)
        ]

    def out_copy(g):
        return pltpu.make_async_copy(obuf.at[g & 1], o_hbm.at[pl.ds(g * G, G)], osem.at[g & 1])

    R0 = PAD + 2
    BR = NB * G
    NS = (H - R0 - 2 * G) // BR
    head = [in_copies(0, R0, 0), in_copies(R0, G, 1), in_copies(R0 + G, G, 2)]

    def block(b):
        return in_copies(R0 + 2 * G + b * BR, BR, 3)

    rest = in_copies(R0 + 2 * G + NS * BR, H - (R0 + 2 * G + NS * BR), 3)
    weights = [
        pltpu.make_async_copy(src, dst, wsem.at[i])
        for i, (src, dst) in enumerate(((dw_hbm, dw_buf), (w1_hbm, w1_buf), (w2t_hbm, w2t_buf)))
    ]
    _start(weights + head[0] + head[1])
    for r0, n in ((SUB, TOP - SUB), (H + TOP, R0 + (NG + 1) * G - H)):
        xbuf[:, pl.ds(r0, n), pl.ds(0, CP), :] = jnp.zeros((NT, n, CP, LANES), jnp.uint32)

    _wait(weights)
    w1 = w1_buf[...].astype(jnp.float32)
    w1 = jnp.concatenate([w1, jnp.zeros((LANES - C, w1.shape[1]), jnp.float32)], axis=0)
    w1t_ref[...] = pltpu.bitcast(_flip(w1.T).astype(jnp.bfloat16), jnp.uint32)
    w2t_ref[...] = pltpu.bitcast(w2t_buf[...], jnp.uint32)

    k = _iota((KS, LANES), 1)
    col = jnp.where(k < KM, k // (2 * SUB), KS - 1 - (k - KM) // 2)
    one_hot = jnp.where(col == _iota((KS, LANES), 0), 1.0, 0.0).astype(jnp.float32)
    for i in range(KS):
        taps_ref[i] = lax.dot_general(
            dw_buf[i].astype(jnp.float32), one_hot, (((0,), (0,)), ((), ())),
            preferred_element_type=jnp.float32)

    def banded(kernel_row, c):
        acc = jnp.zeros(kernel_row.shape, jnp.float32)
        for i in range(KS):
            acc = jnp.where(kernel_row == i, taps_ref[i, pl.ds(c, 1), :], acc)
        return acc

    lane = _iota((SUB, LANES), 1)
    sub = _iota((SUB, LANES), 0)
    zero = jnp.zeros((SUB, LANES), jnp.uint32)

    def left(u, t):
        return u[t - 1] if t > 0 else zero

    def right(u, t):
        return u[t + 1] if t + 1 < NT else zero

    def shifted(main, lead):
        slabs = []
        for d in range(-PAD, PAD + 1):
            r = [pltpu.roll(u, (-d) % LANES, 1) if d else u for u in main]
            if d > 0:
                r = [jnp.where(lane < LANES - d, r[t], right(r, t)) for t in range(NT)]
            elif d < 0:
                r = [jnp.where(lane < -d, left(r, t), r[t]) for t in range(NT)]
            slabs.append(jnp.concatenate(r, axis=1))
        if lead is None:
            slabs.append(jnp.zeros((SUB, W), jnp.uint32))
        else:
            d, src = PAD - sub, (lane + PAD) % LANES
            r = [jnp.broadcast_to(u, (SUB, LANES)) for u in lead]
            r = [jnp.where(src < d, right(r, t), jnp.where(src >= LANES + d, left(r, t), r[t]))
                 for t in range(NT)]
            slabs.append(jnp.concatenate(
                [pltpu.roll(u, 0, 1, stride=1, stride_axis=0) for u in r], axis=1))
        return _bf16(jnp.concatenate(slabs, axis=0))

    def rows8(row0, p):
        return [xflat[t, pl.ds(row0 * XS + p, SUB, stride=XS), :] for t in range(NT)]

    def stage_lead(i, p):
        a, b = ([xbuf[t, i * G + PAD + TOP + e, pl.ds(p, SUB), :] for t in range(NT)]
                for e in range(2))
        for e, halves in enumerate((_low_halves, _high_halves)):
            for t, u in enumerate(halves(a, b)):
                lead_ref[e, t, pl.ds(p, SUB), :] = pltpu.roll(u, LANES - PAD, 1)

    def conv(i, channels):
        results = []
        row0 = i * G + PAD + TOP + 2
        for c in channels:
            p, e = divmod(c, 2)
            if e == 0 or not results:
                a, b = rows8(row0, p), rows8(row0 + SUB, p)
            main = (_low_halves, _high_halves)[e](a, b)
            lead = [lead_ref[e, t, pl.ds(p, 1), :] for t in range(NT)]
            results.append((c, _mm(band_ref[c], shifted(main, lead))))
            if c % (2 * SUB) == 2 * SUB - 1:
                stage_lead(i + 1, p - (SUB - 1))
        return results

    def commit(g, results):
        if not results:
            return
        carried = _iota((SUB, W), 0) >= G - 2 * SUB
        sums = None
        for c, res in results:
            y = jnp.concatenate([carry_ref[c] + res[:SUB], res[SUB:]], axis=0)
            carry_ref[c] = jnp.where(carried, res[2 * SUB:], 0.0)
            for t in range(NT):
                for m0 in range(0, G, SUB):
                    n = min(SUB, G - m0)
                    y_ref[g & 1, t, pl.ds(m0 * YS + c, n, stride=YS), :] = (
                        y[m0:m0 + n, t * LANES:(t + 1) * LANES])
            sums = (y, y * y) if sums is None else (sums[0] + y, sums[1] + y * y)
        if results[0][0] == 0:
            stat_ref[2], stat_ref[3] = sums
        else:
            stat_ref[2] += sums[0]
            stat_ref[3] += sums[1]

    def finish_stats():
        mean = stat_ref[2] * (1.0 / C)
        var = jnp.maximum(stat_ref[3] * (1.0 / C) - mean * mean, 0.0)
        stat_ref[0] = mean
        stat_ref[1] = lax.rsqrt(var + EPS) * _S

    def up(g, r):
        m = (r + 2) % SUB if r < SUB else r
        y = jnp.concatenate([y_ref[g & 1, t, pl.ds(m * YS, C), :] for t in range(NT)], axis=1)
        h = (y - stat_ref[0, pl.ds(m, 1), :]) * stat_ref[1, pl.ds(m, 1), :]
        h = jnp.concatenate([h, jnp.zeros((LANES - C, W), jnp.float32)], axis=0)
        v = _mm(_bf16(w1t_ref[...]), h.astype(jnp.bfloat16))
        th = jnp.tanh(v * (v * v + _A / _S))
        return _flip(v * th + v).astype(jnp.bfloat16)

    def down(g, r, act):
        o = _mm(_bf16(w2t_ref[...]), act)
        x = jnp.concatenate(
            [xbuf[t, g * G + TOP + r, pl.ds(0, CP), :] for t in range(NT)], axis=1)
        obuf[g & 1, r] = (_bf16(x).astype(jnp.float32) + o * (0.5 / _S)).astype(jnp.bfloat16)

    _wait(head[0])
    for p in range(0, CP, SUB):
        stage_lead(0, p)
    m, k = _iota((M, LANES), 0), _iota((M, LANES), 1)
    out_row = jnp.where(m < SUB, (m + SUB - 2) % SUB, m)
    in_row = jnp.where(k < KM, (k % (2 * SUB)) // 2 + SUB * (k % 2) + 2, k % 2)
    kernel_row = in_row + (KS - 1) - out_row
    s = (lane % (2 * SUB)) // 2
    top_kernel_row = s % 4 - 1 - (sub + SUB - 2) % SUB + PAD
    top_channel = (1 - s // 4) * 2 + lane % 2
    for c in range(0, C, 4):
        for e in range(4):
            band_ref[c + e] = banded(kernel_row, c + e)
        band = jnp.concatenate(
            [jnp.where(top_channel == e, banded(top_kernel_row, c + e), 0.0) for e in range(4)],
            axis=0)
        main = [a | pltpu.roll(b, SUB // 2, 0)
                for a, b in zip(rows8(SUB, c // 2), rows8(SUB, c // 2 + 1))]
        res = _mm(band, shifted(main, None))
        for e in range(4):
            carry_ref[c + e] = res[e * SUB:(e + 1) * SUB]

    _wait(head[1])
    _start(head[2])
    commit(0, conv(0, range(C)))
    finish_stats()
    _wait(head[2])

    def step(g):
        pl.when(g >= 2)(lambda: out_copy(g - 2).wait())
        c = 0
        for r, (before, after) in enumerate(zip(CONV_BEFORE, CONV_AFTER)):
            results = conv(g + 1, range(c, c + before))
            act = up(g, r)
            commit(g + 1, results)
            c += before
            commit(g + 1, conv(g + 1, range(c, c + after)))
            c += after
            if r == G - 1:
                finish_stats()
            down(g, r, act)
        out_copy(g).start()

    @pl.loop(0, NS + 2)
    def _(seg):
        pl.when(seg < NS)(lambda: _start(block(seg)))
        pl.when(seg == NS)(lambda: _start(rest))
        pl.loop(jnp.maximum((seg - 1) * NB + 1, 0), jnp.minimum(seg * NB + 1, NG))(step)
        pl.when(seg < NS)(lambda: _wait(block(seg)))
        pl.when(seg == NS)(lambda: _wait(rest))

    out_copy(NG - 2).wait()
    tail = []
    for r0 in range(0, H % G, TR):
        act = up(NG, r0)
        for r in range(r0, r0 + TR):
            nxt = up(NG, r + 1) if r + 1 < r0 + TR else None
            down(NG, r, act)
            act = nxt
        tail.append(pltpu.make_async_copy(
            obuf.at[NG & 1, pl.ds(r0, TR)], o_hbm.at[pl.ds(NG * G + r0, TR)],
            osem.at[2 + len(tail)]))
        tail[-1].start()
    out_copy(NG - 1).wait()
    _wait(tail)


@jax.jit
def pallas_standalone__convnext_block__vision_kernel(
    x: jax.Array,
    dw: jax.Array,
    w1: jax.Array,
    w2: jax.Array,
):
    B, H, W, C = x.shape
    F = w1.shape[1]
    NT = W // LANES
    assert B == 1 and W % LANES == 0 and F % LANES == 0 and x.dtype == jnp.bfloat16
    assert C == sum(CONV_BEFORE) + sum(CONV_AFTER) and H >= 3 * G and H % G % TR == 0
    out = pl.pallas_call(
        _kernel,
        out_shape=jax.ShapeDtypeStruct((H, C, W), x.dtype),
        in_specs=[pl.BlockSpec(memory_space=pl.ANY)] * 4,
        out_specs=pl.BlockSpec(memory_space=pl.ANY),
        scratch_shapes=[
            pltpu.VMEM((NT, (H // G + 1) * G + PAD + TOP + 3, XS, LANES), jnp.uint32),
            pltpu.VMEM((2, G, C, W), jnp.bfloat16),
            pltpu.VMEM(dw.shape, dw.dtype),
            pltpu.VMEM((C, F), w1.dtype),
            pltpu.VMEM((C, F), w2.dtype),
            pltpu.VMEM((F // 2, LANES), jnp.uint32),
            pltpu.VMEM((C // 2, F), jnp.uint32),
            pltpu.VMEM((KS, C, LANES), jnp.float32),
            pltpu.VMEM((C, M, LANES), jnp.float32),
            pltpu.VMEM((2, NT, C // 2, LANES), jnp.uint32),
            pltpu.VMEM((2, NT, (G + 2) * YS, LANES), jnp.float32),
            pltpu.VMEM((C, SUB, W), jnp.float32),
            pltpu.VMEM((4, M, W), jnp.float32),
            pltpu.SemaphoreType.DMA((3,)),
            pltpu.SemaphoreType.DMA((4, NT)),
            pltpu.SemaphoreType.DMA((2 + H % G // TR,)),
        ],
        compiler_params=pltpu.CompilerParams(vmem_limit_bytes=100 * 2**20),
        name="convnext_block",
    )(jnp.transpose(x.reshape(H, W, C), (0, 2, 1)), dw, w1, w2.T)
    return jnp.transpose(out, (0, 2, 1)).reshape(B, H, W, C)
```

```python
import math

import jax
import jax.numpy as jnp
from jax import lax
import jax.experimental.pallas as pl
import jax.experimental.pallas.tpu as pltpu

KS = 7
PAD = KS // 2
SUB = 8
LANES = 128
G = 2 * SUB + 2
M = G + KS - 1
KM = 2 * SUB * KS
XS = 52
YS = 100
NB = 4
TR = 4
EPS = 1e-5
MAX_CANCEL = 256.0
F32_MAX = 3.0e38

CONV_BEFORE = (0,) + (2,) * (G - 1)
CONV_AFTER = (4,) * 8 + (3,) * 10

_A = math.sqrt(2.0 / math.pi)
_S = (_A * 0.044715) ** (1.0 / 3.0)


def _mm(a, b):
    return lax.dot_general(a, b, (((1,), (0,)), ((), ())), preferred_element_type=jnp.float32)


def _bf16(words):
    return pltpu.bitcast(words, jnp.bfloat16)


def _iota(shape, axis):
    return lax.broadcasted_iota(jnp.int32, shape, axis)


def _start(copies):
    for c in copies:
        c.start()


def _wait(copies):
    for c in copies:
        c.wait()


def _low_halves(a, b):
    return [(u & jnp.uint32(0xFFFF)) | (w << 16) for u, w in zip(a, b)]


def _high_halves(a, b):
    return [(u >> 16) | (w & jnp.uint32(0xFFFF0000)) for u, w in zip(a, b)]


def _flip(m):
    order = [i // 8 * 8 + 7 - i % 8 for i in range(m.shape[0] // 16)]
    return jnp.concatenate([m[16 * i:16 * (i + 1)] for i in order], axis=0)


def _kernel(x_hbm, dw_hbm, w1_hbm, w2t_hbm, o_hbm,
            xbuf, obuf, dw_buf, w1_buf, w2t_buf, w1t_ref, w2t_ref, taps_ref, band_ref,
            main_ref, lead_ref, y_ref, carry_ref, stat_ref, wsem, isem, osem):
    H, C, W = x_hbm.shape
    NT = W // LANES
    CP = C // 2
    NG = H // G

    def in_copy(row0, nrows, s):
        return pltpu.make_async_copy(
            x_hbm.at[pl.ds(row0, nrows)], xbuf.at[pl.ds(row0, nrows)], isem.at[s])

    def out_copy(g):
        return pltpu.make_async_copy(obuf.at[g & 1], o_hbm.at[pl.ds(g * G, G)], osem.at[g & 1])

    head = [in_copy(0, PAD, 0)] + [in_copy(PAD + i * G, G, 1 + i) for i in range(3)]
    R0 = PAD + 3 * G
    BR = NB * G
    NS = (H - R0 - 1) // BR

    def block(b):
        return in_copy(R0 + b * BR, BR, 4)

    rest = in_copy(R0 + NS * BR, H - (R0 + NS * BR), 4)
    weights = [
        pltpu.make_async_copy(src, dst, wsem.at[i])
        for i, (src, dst) in enumerate(((dw_hbm, dw_buf), (w1_hbm, w1_buf), (w2t_hbm, w2t_buf)))
    ]
    _start(weights + head[:2])
    xbuf[pl.ds(H, xbuf.shape[0] - H)] = jnp.zeros((xbuf.shape[0] - H, C, W), jnp.bfloat16)

    _wait(weights)
    w1 = w1_buf[...].astype(jnp.float32)
    w1 = jnp.concatenate([w1, jnp.zeros((LANES - C, w1.shape[1]), jnp.float32)], axis=0)
    w1t_ref[...] = pltpu.bitcast(_flip(w1.T).astype(jnp.bfloat16), jnp.uint32)
    w2t_ref[...] = pltpu.bitcast(w2t_buf[...], jnp.uint32)

    k = _iota((KS, LANES), 1)
    col = jnp.where(k < KM, k // (2 * SUB), KS - 1 - (k - KM) // 2)
    one_hot = jnp.where(col == _iota((KS, LANES), 0), 1.0, 0.0).astype(jnp.float32)
    for i in range(KS):
        taps_ref[i] = lax.dot_general(
            dw_buf[i].astype(jnp.float32), one_hot, (((0,), (0,)), ((), ())),
            preferred_element_type=jnp.float32)

    def banded(kernel_row, c):
        acc = jnp.zeros(kernel_row.shape, jnp.float32)
        for i in range(KS):
            acc = jnp.where(kernel_row == i, taps_ref[i, pl.ds(c, 1), :], acc)
        return acc

    lane = _iota((SUB, LANES), 1)
    sub = _iota((SUB, LANES), 0)
    zero = jnp.zeros((SUB, LANES), jnp.uint32)

    def left(u, t):
        return u[t - 1] if t > 0 else zero

    def right(u, t):
        return u[t + 1] if t + 1 < NT else zero

    def shifted(main, lead):
        slabs = []
        for d in range(-PAD, PAD + 1):
            r = [pltpu.roll(u, (-d) % LANES, 1) if d else u for u in main]
            if d > 0:
                r = [jnp.where(lane < LANES - d, r[t], right(r, t)) for t in range(NT)]
            elif d < 0:
                r = [jnp.where(lane < -d, left(r, t), r[t]) for t in range(NT)]
            slabs.append(jnp.concatenate(r, axis=1))
        if lead is None:
            slabs.append(jnp.zeros((SUB, W), jnp.uint32))
        else:
            d, src = PAD - sub, (lane + PAD) % LANES
            r = [jnp.broadcast_to(u, (SUB, LANES)) for u in lead]
            r = [jnp.where(src < d, right(r, t), jnp.where(src >= LANES + d, left(r, t), r[t]))
                 for t in range(NT)]
            slabs.append(jnp.concatenate(
                [pltpu.roll(u, 0, 1, stride=1, stride_axis=0) for u in r], axis=1))
        return _bf16(jnp.concatenate(slabs, axis=0))

    def rows8(row0, p):
        return [main_ref[t, pl.ds(row0 * XS + p, SUB, stride=XS), :] for t in range(NT)]

    def words(h, p):
        w = pltpu.bitcast(xbuf[h, pl.ds(2 * p, 2 * SUB), :], jnp.uint32)
        return [w[:, t * LANES:(t + 1) * LANES] for t in range(NT)]

    def stage(i, p):
        h0 = i * G + PAD
        a, b = words(h0, p), words(h0 + 1, p)
        for e, halves in enumerate((_low_halves, _high_halves)):
            for t, u in enumerate(halves(a, b)):
                lead_ref[e, t, pl.ds(p, SUB), :] = pltpu.roll(u, LANES - PAD, 1)
        for r in range(2 * SUB):
            for t, u in enumerate(words(h0 + 2 + r, p)):
                main_ref[t, pl.ds(r * XS + p, SUB), :] = u

    def conv(i, channels, restage=True):
        results = []
        for c in channels:
            p, e = divmod(c, 2)
            if e == 0 or not results:
                a, b = rows8(0, p), rows8(SUB, p)
            main = (_low_halves, _high_halves)[e](a, b)
            lead = [lead_ref[e, t, pl.ds(p, 1), :] for t in range(NT)]
            results.append((c, _mm(band_ref[c], shifted(main, lead))))
            if restage and c % (2 * SUB) == 2 * SUB - 1:
                stage(jnp.minimum(i + 1, NG), p - (SUB - 1))
        return results

    def commit(g, results):
        if not results:
            return
        carried = _iota((SUB, W), 0) >= G - 2 * SUB
        sums = None
        for c, res in results:
            y = jnp.concatenate([carry_ref[c] + res[:SUB], res[SUB:]], axis=0)
            carry_ref[c] = jnp.where(carried, res[2 * SUB:], 0.0)
            for t in range(NT):
                for m0 in range(0, G, SUB):
                    n = min(SUB, G - m0)
                    y_ref[g & 1, t, pl.ds(m0 * YS + c, n, stride=YS), :] = (
                        y[m0:m0 + n, t * LANES:(t + 1) * LANES])
            sums = (y, y * y) if sums is None else (sums[0] + y, sums[1] + y * y)
        if results[0][0] == 0:
            stat_ref[2], stat_ref[3] = sums
        else:
            stat_ref[2] += sums[0]
            stat_ref[3] += sums[1]

    def finish_stats():
        mean = stat_ref[2] * (1.0 / C)
        var = jnp.maximum(stat_ref[3] * (1.0 / C) - mean * mean, 0.0) + EPS
        stat_ref[0] = mean
        stat_ref[1] = lax.rsqrt(var) * _S
        safe = (mean * mean <= MAX_CANCEL * var) & (var <= F32_MAX)
        return jnp.max(jnp.where(safe | (_iota((M, W), 0) >= G), 0.0, 1.0)) > 0.0

    def centred_stats(g):
        stat_ref[3] = jnp.zeros((M, W), jnp.float32)

        @pl.loop(0, C)
        def _(c):
            for t in range(NT):
                for m0 in range(0, G, SUB):
                    n = min(SUB, G - m0)
                    at = (pl.ds(m0, n), pl.ds(t * LANES, LANES))
                    d = y_ref[g & 1, t, pl.ds(m0 * YS + c, n, stride=YS), :] - stat_ref[(0,) + at]
                    stat_ref[(3,) + at] += d * d

        stat_ref[1] = lax.rsqrt(stat_ref[3] * (1.0 / C) + EPS) * _S

    def up(g, r):
        m = (r + 2) % SUB if r < SUB else r
        y = jnp.concatenate([y_ref[g & 1, t, pl.ds(m * YS, C), :] for t in range(NT)], axis=1)
        h = (y - stat_ref[0, pl.ds(m, 1), :]) * stat_ref[1, pl.ds(m, 1), :]
        h = jnp.concatenate([h, jnp.zeros((LANES - C, W), jnp.float32)], axis=0)
        v = _mm(_bf16(w1t_ref[...]), h.astype(jnp.bfloat16))
        th = jnp.tanh(v * (v * v + _A / _S))
        return _flip(v * th + v).astype(jnp.bfloat16)

    def down(g, r, act):
        o = _mm(_bf16(w2t_ref[...]), act)
        x = xbuf[g * G + r].astype(jnp.float32)
        obuf[g & 1, r] = (x + o * (0.5 / _S)).astype(jnp.bfloat16)

    head[0].wait()
    for r in range(SUB):
        for p in range(0, CP, SUB):
            w = words(r - (SUB - PAD), p) if r >= SUB - PAD else [zero] * NT
            for t in range(NT):
                main_ref[t, pl.ds(r * XS + p, SUB), :] = w[t]
    m, k = _iota((M, LANES), 0), _iota((M, LANES), 1)
    out_row = jnp.where(m < SUB, (m + SUB - 2) % SUB, m)
    in_row = jnp.where(k < KM, (k % (2 * SUB)) // 2 + SUB * (k % 2) + 2, k % 2)
    kernel_row = in_row + (KS - 1) - out_row
    s = (lane % (2 * SUB)) // 2
    top_kernel_row = s % 4 - 1 - (sub + SUB - 2) % SUB + PAD
    top_channel = (1 - s // 4) * 2 + lane % 2
    for c in range(0, C, 4):
        for e in range(4):
            band_ref[c + e] = banded(kernel_row, c + e)
        band = jnp.concatenate(
            [jnp.where(top_channel == e, banded(top_kernel_row, c + e), 0.0) for e in range(4)],
            axis=0)
        main = [a | pltpu.roll(b, SUB // 2, 0)
                for a, b in zip(rows8(0, c // 2), rows8(0, c // 2 + 1))]
        res = _mm(band, shifted(main, None))
        for e in range(4):
            carry_ref[c + e] = res[e * SUB:(e + 1) * SUB]

    head[1].wait()
    _start(head[2:])
    for p in range(0, CP, SUB):
        stage(0, p)
    commit(0, conv(0, range(C), restage=False))
    pl.when(finish_stats())(lambda: centred_stats(0))
    head[2].wait()
    for p in range(0, CP, SUB):
        stage(1, p)
    head[3].wait()

    def step(g):
        pl.when(g >= 2)(lambda: out_copy(g - 2).wait())
        c = 0
        for r, (before, after) in enumerate(zip(CONV_BEFORE, CONV_AFTER)):
            results = conv(g + 1, range(c, c + before))
            act = up(g, r)
            commit(g + 1, results)
            c += before
            commit(g + 1, conv(g + 1, range(c, c + after)))
            c += after
            if r == G - 1:
                unsafe = finish_stats()
            down(g, r, act)
        out_copy(g).start()
        pl.when(unsafe)(lambda: centred_stats(g + 1))

    @pl.loop(0, NS + 2)
    def _(seg):
        pl.when(seg < NS)(lambda: block(seg).start())
        pl.when(seg == NS)(rest.start)
        pl.loop(jnp.maximum((seg - 1) * NB + 1, 0), jnp.minimum(seg * NB + 1, NG))(step)
        pl.when(seg < NS)(lambda: block(seg).wait())
        pl.when(seg == NS)(rest.wait)

    out_copy(NG - 2).wait()
    tail = []
    for r0 in range(0, H % G, TR):
        act = up(NG, r0)
        for r in range(r0, r0 + TR):
            nxt = up(NG, r + 1) if r + 1 < r0 + TR else None
            down(NG, r, act)
            act = nxt
        tail.append(pltpu.make_async_copy(
            obuf.at[NG & 1, pl.ds(r0, TR)], o_hbm.at[pl.ds(NG * G + r0, TR)],
            osem.at[2 + len(tail)]))
        tail[-1].start()
    out_copy(NG - 1).wait()
    _wait(tail)


@jax.jit
def pallas_standalone__convnext_block__vision_kernel(
    x: jax.Array,
    dw: jax.Array,
    w1: jax.Array,
    w2: jax.Array,
):
    B, H, W, C = x.shape
    F = w1.shape[1]
    NT = W // LANES
    assert B == 1 and W % LANES == 0 and F % LANES == 0 and x.dtype == jnp.bfloat16
    assert C == sum(CONV_BEFORE) + sum(CONV_AFTER) and H > PAD + 3 * G and H % G % TR == 0
    out = pl.pallas_call(
        _kernel,
        out_shape=jax.ShapeDtypeStruct((H, C, W), x.dtype),
        in_specs=[pl.BlockSpec(memory_space=pl.ANY)] * 4,
        out_specs=pl.BlockSpec(memory_space=pl.ANY),
        scratch_shapes=[
            pltpu.VMEM(((H // G + 1) * G + PAD, C, W), jnp.bfloat16),
            pltpu.VMEM((2, G, C, W), jnp.bfloat16),
            pltpu.VMEM(dw.shape, dw.dtype),
            pltpu.VMEM((C, F), w1.dtype),
            pltpu.VMEM((C, F), w2.dtype),
            pltpu.VMEM((F // 2, LANES), jnp.uint32),
            pltpu.VMEM((C // 2, F), jnp.uint32),
            pltpu.VMEM((KS, C, LANES), jnp.float32),
            pltpu.VMEM((C, M, LANES), jnp.float32),
            pltpu.VMEM((NT, G * XS, LANES), jnp.uint32),
            pltpu.VMEM((2, NT, C // 2, LANES), jnp.uint32),
            pltpu.VMEM((2, NT, (G + 2) * YS, LANES), jnp.float32),
            pltpu.VMEM((C, SUB, W), jnp.float32),
            pltpu.VMEM((4, M, W), jnp.float32),
            pltpu.SemaphoreType.DMA((3,)),
            pltpu.SemaphoreType.DMA((5,)),
            pltpu.SemaphoreType.DMA((2 + H % G // TR,)),
        ],
        compiler_params=pltpu.CompilerParams(vmem_limit_bytes=80 * 2**20),
        name="convnext_block",
    )(jnp.transpose(x.reshape(H, W, C), (0, 2, 1)), dw, w1, w2.T)
    return jnp.transpose(out, (0, 2, 1)).reshape(B, H, W, C)
```
